```python
import os as _os
_os.environ.setdefault("JAX_PLATFORMS", "cpu")
import jax
import jax.numpy as jnp

def _softmax(x, axis=-1):
    return jax.nn.softmax(x, axis=axis)
def _gelu(x):
    return jax.nn.gelu(x, approximate=True)
def _silu(x):
    return jax.nn.silu(x)
def _sigmoid(x):
    return jax.nn.sigmoid(x)
def _layernorm(x, axis=-1, eps=1e-5):
    m = jnp.mean(x, axis=axis, keepdims=True)
    v = jnp.var(x, axis=axis, keepdims=True)
    return (x - m) / jnp.sqrt(v + eps)
def _scatter_add(tgt, idx, src, axis=0):
    return tgt.at[idx].add(src)
def _segment_sum(src, seg, n):
    return jax.ops.segment_sum(src, seg, n)
class _Rng:
    def __init__(self, key):
        self._k = key
    def _next(self):
        self._k, sub = jax.random.split(self._k)
        return sub
    def normal(self, shape):
        return jax.random.normal(self._next(), shape, dtype=jnp.bfloat16)
    def randint(self, lo, hi, shape):
        return jax.random.randint(self._next(), shape, lo, hi, dtype=jnp.int32)
    def uniform(self, shape, lo=0.0, hi=1.0):
        return jax.random.uniform(self._next(), shape, jnp.bfloat16, lo, hi)
    def permutation(self, n):
        return jax.random.permutation(self._next(), n)


kernel_name = 'standalone__gqa_block_cached__near_ridge'

def setup_inputs():
    _rng = _Rng(jax.random.key(int.from_bytes(__import__("os").urandom(4), "little")))
    _w = (lambda a: (lambda t: t.astype(jnp.bfloat16) if jnp.issubdtype(t.dtype, jnp.floating) else t)(jnp.asarray(a)))
    B, Sq, D = 8, 240, 640
    Hq, Hkv, Sk, Dh = 32, 32, 1024, 192
    assert Hq % Hkv == 0, (Hq, Hkv)
    return {
        "x": _w((lambda *s: _rng.normal(s) * 0.8)(B, Sq, D)),
        "k_cache": _w((lambda *s: _rng.normal(s) * 0.8)(B, Hkv, Sk, Dh)),
        "v_cache": _w((lambda *s: _rng.normal(s) * 0.05)(B, Hkv, Sk, Dh)),
        "wq": _w((lambda *s: _rng.normal(s) * 0.8)(D, Hq * Dh) * (D ** -0.5)),
        "wo": _w((lambda *s: _rng.normal(s) * 0.05)(Hq * Dh, D) * ((Hq * Dh) ** -0.5)),
    }

def reference(x, k_cache, v_cache, wq, wo):
    B, Sq, D = x.shape
    Hq, Dh = 32, 192
    Hkv = k_cache.shape[1]
    rep = Hq // Hkv
    q = (lambda x, *d: x.transpose(*d))((x @ wq).reshape(B, Sq, Hq, Dh), 0, 2, 1, 3)
    k = jnp.repeat(k_cache, rep, axis=1)
    v = jnp.repeat(v_cache, rep, axis=1)
    scores = jnp.einsum("bhqd,bhkd->bhqk", q, k) * (Dh ** -0.5)
    p = _softmax(scores, axis=-1)
    o = jnp.einsum("bhqk,bhkd->bhqd", p, v)
    return (lambda x, *d: x.transpose(*d))(o, 0, 2, 1, 3).reshape(B, Sq, Hq * Dh) @ wo
```

```python
import functools, math
import jax, jax.numpy as jnp
from jax import lax
import jax.experimental.pallas as pl
import jax.experimental.pallas.tpu as pltpu

NT = (((1,), (1,)), ((), ()))
f32 = jnp.float32
bf16 = jnp.bfloat16
u32 = jnp.uint32

def pk(v):
    return pltpu.bitcast(v, u32)
def upk(v):
    return pltpu.bitcast(v, bf16)

def make(NB=4, qkn=256, lag=4, lag_first=5, lag_last=6, tailsplit=0, nfine=2, nobc=True, flagA=6, skipB5=True, Pn=None, pfj=2, sv=3, lowp=0, nosc=True):
    A = lambda i: (0, i)
    Bq = lambda i: (1, i)
    sched = {
        0: [[A(0), A(1)], [A(2)], [A(3)], [A(4)], [Bq(0), Bq(1)], [Bq(2), Bq(3)], [Bq(4)], [], [], [], []],
        1: [[A(0)], [A(1)], [A(2), A(3)], [A(4)], [Bq(0), Bq(1)], [Bq(2), Bq(3)], [Bq(4)], [], [], [], []],
        2: [[A(0), A(1)], [A(2)], [A(3)], [A(4), Bq(0), Bq(1)], [Bq(2), Bq(3)], [Bq(4)], [], [], [], [], []],
        3: [[A(0), A(1), A(2), A(3), A(4), Bq(0), Bq(1), Bq(2), Bq(3), Bq(4)]] + [[]] * 10,
    }[sv]
    @jax.jit
    def fn(x, k_cache, v_cache, wq, wo):
        B, Sq, D = x.shape
        _, H, Sk, Dh = k_cache.shape
        P = H // 2
        W = 2 * Dh
        G = B // NB
        assert G == 2 and nfine in (0, 2)
        Sh = Sq // 2
        kt = jnp.swapaxes(k_cache, 2, 3).reshape(B, P, W, Sk)
        vt = jnp.swapaxes(v_cache, 2, 3).reshape(B, P, W, Sk)
        P = Pn or P
        NSTEP = P * G
        c = (Dh ** -0.5) * math.log2(math.e)

        def kern(x_hbm, kt_hbm, vt_hbm, wq_hbm, wo_hbm, o_hbm,
                 x_ref, kbuf, vbuf, wqbuf, wobuf, obuf, acc_ref,
                 s0, s1, p0, p1, r_sc, ot_sc, sems):
            xsem, k0sem, v0sem, wqsem, wosem, ksem, vsem, osem = 0, 8, 16, 24, 26, 28, 31, 34
            s_sc = (s0, s1); p_sc = (p0, p1)
            p = pl.program_id(0)
            g = pl.program_id(1)
            step = p * G + g
            z1 = p // 1024
            z2 = g // 1024
            z3 = (p + g) // 1024
            never = z1 > 0
            lane = lax.broadcasted_iota(jnp.int32, (Sq, 128), 1)
            lo = lane < 64
            ws = p % 2
            slot = step % 3

            def kv_copy(hbm, buf, sem, pp, gg, sl):
                return pltpu.make_async_copy(hbm.at[pl.ds(gg * NB, NB), pp], buf.at[sl], sems.at[sem + sl])
            def kv_fine(hbm, buf, sem, gg, j):
                return pltpu.make_async_copy(hbm.at[gg * NB + j, 0], buf.at[gg, j], sems.at[sem + gg * NB + j])
            def x_copy(b):
                return pltpu.make_async_copy(x_hbm.at[b], x_ref.at[b], sems.at[xsem + b])
            def wq_copy(pp, sl):
                return pltpu.make_async_copy(wq_hbm.at[:, pl.ds(pl.multiple_of(pp * W, 128), W)], wqbuf.at[sl], sems.at[wqsem + sl])
            def wo_copy(pp, sl):
                return pltpu.make_async_copy(wo_hbm.at[pl.ds(pl.multiple_of(pp * W, 128), W), :], wobuf.at[sl], sems.at[wosem + sl])
            def o_copy(b):
                return pltpu.make_async_copy(obuf.at[b], o_hbm.at[b], sems.at[osem + b])

            def grp(gg, i):
                K = lambda j: kv_fine(kt_hbm, kbuf, k0sem, gg, j)
                V = lambda j: kv_fine(vt_hbm, vbuf, v0sem, gg, j)
                X = lambda j: x_copy(gg * NB + j)
                if i == 0:
                    return ([wq_copy(0, 0)] if gg == 0 else []) + [X(0)]
                if i == 1:
                    return [K(0), X(1)]
                if i == 2:
                    return [V(0), K(1), X(2)]
                if i == 3:
                    return ([wo_copy(0, 0)] if gg == 0 else []) + [V(1), K(2), X(3)]
                return [V(2), K(3), V(3)]
            allg = [(gg, i) for gg in range(2) for i in range(5)]
            def start_groups(lst):
                for gg, i in lst:
                    for cp in grp(gg, i):
                        cp.start(priority=0 if (gg, i) == (0, 0) else lowp)

            @pl.when(step == 0)
            def _():
                start_groups(sched[0])

            def when(cond, f):
                pl.when(cond)(f)

            def qproj(j):
                q = jnp.dot(x_ref[g * NB + j], wqbuf[ws], preferred_element_type=f32) * c
                q1 = q[:, 128:256]
                qa = jnp.concatenate([q[:, 0:128], jnp.where(lo, q1, 0.0)], axis=1).astype(bf16)
                qb = jnp.concatenate([jnp.where(lo, 0.0, q1), q[:, 256:384]], axis=1).astype(bf16)
                return qa, qb

            def qk(j, h, q):
                u = 2 * j + h
                ss = s_sc[u % 2].at[z1]
                for n in range(Sk // qkn):
                    ss[:, n * qkn:(n + 1) * qkn] = jnp.dot(q, kbuf[slot, j, h * 128:h * 128 + 256, n * qkn:(n + 1) * qkn], preferred_element_type=f32)

            def soft(j, h, lg):
                u = 2 * j + h
                ss = s_sc[u % 2].at[z2]
                sm = s_sc[u % 2].at[z3]
                ps = p_sc[u % 2].at[z1]
                rc = 16
                ms = [jnp.max(sm[i * rc:(i + 1) * rc, :], axis=1, keepdims=True) for i in range(Sq // rc)]
                ls = []
                for i in range(Sq // rc):
                    s = ss[i * rc:(i + 1) * rc, :]
                    m = ms[i]
                    es = []; lss = []
                    for gi in range(rc // 8):
                        mg = m[gi * 8:(gi + 1) * 8]
                        if len(ls) >= lg:
                            mg = jnp.where(never, ls[len(ls) - lg], mg)
                        eg = jnp.exp2(s[gi * 8:(gi + 1) * 8] - mg)
                        lgv = jnp.sum(eg, axis=1, keepdims=True)
                        ls.append(lgv); lss.append(lgv); es.append(eg)
                    e = jnp.concatenate(es, axis=0)
                    l = jnp.concatenate(lss, axis=0)
                    r = pl.reciprocal(l, approx=True)
                    ps[i * rc // 2:(i + 1) * rc // 2, 0:Sk] = pk(e.astype(bf16))
                    ps[Sh + i * rc:Sh + (i + 1) * rc, 0:128] = pltpu.bitcast(jnp.broadcast_to(r, (rc, 128)), u32)

            def pv(j, h):
                u = 2 * j + h
                ps = p_sc[u % 2].at[z2]
                ot_sc[j % 2, h * 64:(h + 1) * 64, :] = lax.dot_general(vbuf[slot, j, 128 + 64 * h:192 + 64 * h, :], upk(ps[0:Sh, :]), NT, preferred_element_type=f32)
                on = lax.dot_general(upk(ps[0:Sh, :]), vbuf[slot, j, 256 * h:256 * h + 128, :], NT, preferred_element_type=f32)
                rr = pltpu.bitcast(ps[Sh:Sh + Sq, 0:128], f32)
                r_sc[u % 4] = rr
                return on * rr

            def omid(j):
                o1 = ot_sc[j % 2].T
                return o1 * jnp.where(lo, r_sc[(2 * j) % 4], r_sc[(2 * j + 1) % 4])

            def oproj(j, o, first, n0=0, n1=D, fin=True):
                b = g * NB + j
                y = jnp.dot(o, wobuf[ws, :, n0:n1], preferred_element_type=f32)
                if first is None:
                    y = y + jnp.where(p > 0, acc_ref[b, :, n0:n1], 0.0)
                elif not first:
                    y = y + acc_ref[b, :, n0:n1]
                acc_ref[b, :, n0:n1] = y
                if first is not True:
                    obuf[b, :, n0:n1] = y.astype(bf16)
                    if fin:
                        when(p == P - 1, lambda: o_copy(b).start())

            def body(fine):
                first = (True if fine else False) if nfine else None
                def barrier(i):
                    for gg in range(2):
                        def f(gg=gg):
                            for cp in grp(gg, i):
                                cp.wait()
                            start_groups(sched[1 + gg * 5 + i])
                        when(g == gg, f)
                if fine:
                    barrier(0)
                else:
                    if nfine == 0:
                        @pl.when(p == 0)
                        def _():
                            for j in range(NB):
                                x_copy(g * NB + j).wait()
                                kv_fine(kt_hbm, kbuf, k0sem, g, j).wait()
                                kv_fine(vt_hbm, vbuf, v0sem, g, j).wait()
                        when(p > 0, lambda: kv_copy(kt_hbm, kbuf, ksem, p, g, slot).wait())
                        when(p > 0, lambda: kv_copy(vt_hbm, vbuf, vsem, p, g, slot).wait())
                    else:
                        kv_copy(kt_hbm, kbuf, ksem, p, g, slot).wait()
                        kv_copy(vt_hbm, vbuf, vsem, p, g, slot).wait()
                    when(g == 0, lambda: wq_copy(p, ws).wait())
                    when(g == 0, lambda: wo_copy(p, ws).wait())

                def prefetch():
                    pn = jnp.minimum(p + 1, P - 1)
                    sn = (step + 2) % 3
                    when(jnp.logical_and(g == 0, p + 1 < P), lambda: wq_copy(pn, 1 - ws).start())
                    when(p + 1 < P, lambda: kv_copy(kt_hbm, kbuf, ksem, pn, g, sn).start(priority=lowp))
                    when(p + 1 < P, lambda: kv_copy(vt_hbm, vbuf, vsem, pn, g, sn).start(priority=lowp))
                    when(jnp.logical_and(g == 0, p + 1 < P), lambda: wo_copy(pn, 1 - ws).start())
                if not fine:
                    prefetch()

                q = {}; on = {}; o = {}
                q[0] = qproj(0)
                if fine:
                    barrier(1)
                for j in range(NB):
                    qk(j, 0, q[j][0])
                    soft(j, 0, lag_first if j == 0 else (flagA if fine and j == NB - 1 and not skipB5 else lag))
                    if j + 1 < NB:
                        q[j + 1] = qproj(j + 1)
                    if j > 0:
                        on[j - 1, 1] = pv(j - 1, 1)
                        o[j - 1] = jnp.concatenate([on[j - 1, 0], omid(j - 1), on[j - 1, 1]], axis=1).astype(bf16)
                    qk(j, 1, q[j][1])
                    if fine and j < NB - 1:
                        barrier(j + 2)
                        if j == pfj:
                            prefetch()
                    soft(j, 1, lag_last if j == NB - 1 else lag)
                    if j > 0:
                        if tailsplit and j == NB - 1:
                            oproj(j - 1, o[j - 1], first, 0, D - tailsplit, fin=False)
                        else:
                            oproj(j - 1, o[j - 1], first)
                    on[j, 0] = pv(j, 0)
                j = NB - 1
                on[j, 1] = pv(j, 1)
                if tailsplit:
                    oproj(j - 1, o[j - 1], first, D - tailsplit, D)
                o[j] = jnp.concatenate([on[j, 0], omid(j), on[j, 1]], axis=1).astype(bf16)
                oproj(j, o[j], first)

            if nfine:
                pl.when(p == 0)(lambda: body(True))
                pl.when(p > 0)(lambda: body(False))
            else:
                body(False)

            @pl.when(step == NSTEP - 1)
            def _():
                for b in range(B):
                    o_copy(b).wait()

        out = pl.pallas_call(
            kern,
            grid=(P, G),
            in_specs=[pl.BlockSpec(memory_space=pl.ANY)] * 5,
            out_specs=pl.BlockSpec(memory_space=pl.ANY),
            out_shape=jax.ShapeDtypeStruct((B, Sq, D), x.dtype),
            scratch_shapes=[
                pltpu.VMEM((B, Sq, D), bf16),
                pltpu.VMEM((3, NB, W, Sk), bf16),
                pltpu.VMEM((3, NB, W, Sk), bf16),
                pltpu.VMEM((2, D, W), bf16),
                pltpu.VMEM((2, W, D), bf16),
                pltpu.VMEM((B, Sq, D), bf16),
                pltpu.VMEM((B, Sq, D), f32),
                pltpu.VMEM((1, Sq, Sk), f32), pltpu.VMEM((1, Sq, Sk), f32),
                pltpu.VMEM((1, Sh + Sq, Sk), u32), pltpu.VMEM((1, Sh + Sq, Sk), u32),
                pltpu.VMEM((4, Sq, 128), f32), pltpu.VMEM((2, 128, Sq), f32),
                pltpu.SemaphoreType.DMA((42,)),
            ],
            compiler_params=pltpu.CompilerParams(dimension_semantics=("arbitrary", "arbitrary"), vmem_limit_bytes=100 * 1024 * 1024,
                                                 disable_bounds_checks=nobc, disable_semaphore_checks=nosc),
        )(x, kt, vt, wq, wo)
        return out
    return fn


_impl = make()


@jax.jit
def pallas_standalone__gqa_block_cached__near_ridge_kernel(x, k_cache, v_cache, wq, wo):
    return _impl(x, k_cache, v_cache, wq, wo)
```

```python
import math

import jax
import jax.numpy as jnp
from jax import lax
import jax.experimental.pallas as pl
import jax.experimental.pallas.tpu as pltpu

_NT = (((1,), (1,)), ((), ()))
_F32 = jnp.float32
_BF16 = jnp.bfloat16
_U32 = jnp.uint32

_NB = 4
_NSL = 4
_LAGS = (5, 4, 4, 4, 4, 4, 4, 7)
_MPACE = 4
_CUT = 0.3


def _pk(v):
    return pltpu.bitcast(v, _U32)


def _upk(v):
    return pltpu.bitcast(v, _BF16)


def _dot(a, b):
    return jnp.dot(a, b, preferred_element_type=_F32)


def _dot_nt(a, b):
    return lax.dot_general(a, b, _NT, preferred_element_type=_F32)


@jax.jit
def pallas_standalone__gqa_block_cached__near_ridge_kernel(
    x: jax.Array,
    k_cache: jax.Array,
    v_cache: jax.Array,
    wq: jax.Array,
    wo: jax.Array,
):
    B, Sq, D = x.shape
    _, H, Sk, Dh = k_cache.shape
    NB, NSL = _NB, _NSL
    P = H // 2
    W = 2 * Dh
    assert B == 2 * NB and Dh == 192 and wq.shape == (D, H * Dh) and Sq == 240
    Sh = Sq // 2
    NG = Sq // 8
    NSTEP = 2 * P
    kt = jnp.swapaxes(k_cache, 2, 3).reshape(B, P, W, Sk)
    vt = jnp.swapaxes(v_cache, 2, 3).reshape(B, P, W, Sk)
    qscale = (Dh ** -0.5) * math.log2(math.e)

    def kern(x_hbm, kt_hbm, vt_hbm, wq_hbm, wo_hbm, o_hbm,
             x_ref, kbuf, vbuf, wqbuf, wobuf, obuf, acc_ref,
             s0, s1, p0, p1, r_sc, ot0, ot1, sems):
        xsem, k0sem, v0sem, wqsem, wosem, ksem, vsem, osem = 0, 8, 16, 24, 26, 28, 32, 36
        s_sc, p_sc, ot_sc = (s0, s1), (p0, p1), (ot0, ot1)
        lo = lax.broadcasted_iota(jnp.int32, (Sq, 128), 1) < 64

        def kv_copy(hbm, buf, sem, st):
            sl = st & (NSL - 1)
            return pltpu.make_async_copy(hbm.at[pl.ds((st & 1) * NB, NB), st >> 1],
                                         buf.at[pl.ds(sl * NB, NB)], sems.at[sem + sl])

        def k0_copy(b):
            return pltpu.make_async_copy(kt_hbm.at[b, 0], kbuf.at[b], sems.at[k0sem + b])

        def v0_copy(b):
            return pltpu.make_async_copy(vt_hbm.at[b, 0], vbuf.at[b], sems.at[v0sem + b])

        def x_copy(b):
            return pltpu.make_async_copy(x_hbm.at[b], x_ref.at[b], sems.at[xsem + b])

        def wq_copy(pp):
            return pltpu.make_async_copy(wq_hbm.at[:, pl.ds(pl.multiple_of(pp * W, 128), W)],
                                         wqbuf.at[pp & 1], sems.at[wqsem + (pp & 1)])

        def wo_copy(pp):
            return pltpu.make_async_copy(wo_hbm.at[pl.ds(pl.multiple_of(pp * W, 128), W), :],
                                         wobuf.at[pp & 1], sems.at[wosem + (pp & 1)])

        def o_copy(b):
            return pltpu.make_async_copy(obuf.at[b], o_hbm.at[b], sems.at[osem + b])

        groups = (((x_copy, 0),),
                  ((k0_copy, 0), (x_copy, 1)),
                  ((v0_copy, 0), (k0_copy, 1), (x_copy, 2)),
                  ((v0_copy, 1), (k0_copy, 2), (x_copy, 3)),
                  ((v0_copy, 2), (k0_copy, 3), (v0_copy, 3)))

        def on_even(st, f):
            if isinstance(st, int):
                if st % 2 == 0:
                    f()
            else:
                pl.when((st & 1) == 0)(f)

        def prefetch(st):
            on_even(st, lambda: wq_copy(st >> 1).start())
            kv_copy(kt_hbm, kbuf, ksem, st).start()
            kv_copy(vt_hbm, vbuf, vsem, st).start()
            on_even(st, lambda: wo_copy(st >> 1).start())

        def run(mode, step):
            first = mode == 'first'
            z1 = lax.shift_right_logical(step, 10)
            z2 = lax.shift_right_logical(step, 11)
            z3 = lax.shift_right_logical(step, 12)
            never = z1 > 0
            if first:
                ws, b0, kv0 = 0, step * NB, step * NB
            else:
                ws = (step >> 1) & 1
                b0 = (step & 1) * NB
                kv0 = (step & (NSL - 1)) * NB

            def rows_dot(lhs, rhs):
                if first:
                    return jnp.concatenate([_dot(lhs[0:128], rhs), _dot(lhs[128:Sq], rhs)], axis=0)
                return _dot(lhs, rhs)

            def qproj(j):
                q = rows_dot(x_ref[b0 + j], wqbuf[ws]) * qscale
                q1 = q[:, 128:256]
                qa = jnp.concatenate([q[:, 0:128], jnp.where(lo, q1, 0.0)], axis=1).astype(_BF16)
                qb = jnp.concatenate([jnp.where(lo, 0.0, q1), q[:, 256:384]], axis=1).astype(_BF16)
                return (qa, qb), [(q, r, c * 128) for c in range(3) for r in range(NG)]

            def qk(j, h, q):
                ss = s_sc[h].at[z1]
                ticks = []
                for n in range(Sk // 256):
                    sv = _dot(q, kbuf[kv0 + j, h * 128:h * 128 + 256, n * 256:(n + 1) * 256])
                    ss[:, n * 256:(n + 1) * 256] = sv
                    ticks += [(sv, r, 0) for r in range(NG)]
                return ticks

            def soft(j, h, ticks=None):
                ss = s_sc[h].at[z2]
                sm = s_sc[h].at[z3]
                ps = p_sc[h].at[z1]

                def tick(g):
                    sv, r, c = ticks[int(g * len(ticks) / NG)]
                    return sv[r * 8:(r + 1) * 8, c:c + 128]

                ms = []
                if ticks is not None:
                    for g in range(NG):
                        sv8 = sm[g * 8:(g + 1) * 8, :]
                        t0 = sv8[:, 0:128]
                        if g >= _MPACE:
                            t0 = jnp.where(never, tick(g - _MPACE), t0)
                        for t in range(1, Sk // 128):
                            t0 = jnp.maximum(t0, sv8[:, t * 128:(t + 1) * 128])
                        ms.append(jnp.max(t0, axis=1, keepdims=True))
                else:
                    for i in range(NG // 2):
                        m = jnp.max(sm[i * 16:(i + 1) * 16, :], axis=1, keepdims=True)
                        ms += [m[0:8], m[8:16]]
                ls = []
                for i in range(NG // 2):
                    s = ss[i * 16:(i + 1) * 16, :]
                    es = []
                    for gi in range(2):
                        g = 2 * i + gi
                        sg = s[gi * 8:(gi + 1) * 8]
                        if ticks is not None:
                            mb = jnp.where(never, tick(g), jnp.broadcast_to(ms[g], (8, 128)))
                            eg = jnp.concatenate(
                                [jnp.exp2(sg[:, t * 128:(t + 1) * 128] - mb) for t in range(Sk // 128)], axis=1)
                        else:
                            lag = _LAGS[2 * j + h]
                            mg = jnp.where(never, ls[g - lag], ms[g]) if g >= lag else ms[g]
                            eg = jnp.exp2(sg - mg)
                        ls.append(jnp.sum(eg, axis=1, keepdims=True))
                        es.append(eg)
                    ps[i * 8:(i + 1) * 8, :] = _pk(jnp.concatenate(es, axis=0).astype(_BF16))
                    if ticks is not None:
                        for g in (2 * i, 2 * i + 1):
                            ps[Sh + g * 8:Sh + (g + 1) * 8, 0:128] = _pk(jnp.broadcast_to(ls[g], (8, 128)))
                    else:
                        l = jnp.concatenate(ls[-2:], axis=0)
                        ps[Sh + i * 16:Sh + (i + 1) * 16, 0:128] = _pk(jnp.broadcast_to(l, (16, 128)))

            def pv(j, h):
                ps = p_sc[h].at[z2]
                ot = on = None
                ticks = []
                for kc in range(Sk // 128):
                    k0, k1 = kc * 128, (kc + 1) * 128
                    a = _dot_nt(vbuf[kv0 + j, 128 + 64 * h:192 + 64 * h, k0:k1], _upk(ps[0:Sh, k0:k1]))
                    ot = a if ot is None else ot + a
                    if kc == Sk // 128 - 1:
                        ot_sc[j % 2].at[z1][h * 64:(h + 1) * 64, :] = ot
                    a = _dot_nt(_upk(ps[0:Sh, k0:k1]), vbuf[kv0 + j, 256 * h:256 * h + 128, k0:k1])
                    on = a if on is None else on + a
                    ticks += [(a, r, 0) for r in range(12)]
                rr = 1.0 / pltpu.bitcast(ps[Sh:Sh + Sq, 0:128], _F32)
                r_sc[(2 * j + h) % 4] = rr
                return on * rr, ticks

            def omid(j):
                o1 = ot_sc[j % 2].at[z2][...].T
                return o1 * jnp.where(lo, r_sc[(2 * j) % 4], r_sc[(2 * j + 1) % 4])

            def oproj(j, o, split=False):
                b = b0 + j
                y = None if first else acc_ref[b]
                if split:
                    for t in (0, 2, 1):
                        yt = _dot(o[t].astype(_BF16), wobuf[ws, t * 128:(t + 1) * 128, :])
                        y = yt if y is None else y + yt
                else:
                    yt = rows_dot(jnp.concatenate(o, axis=1).astype(_BF16), wobuf[ws])
                    y = yt if y is None else yt + y
                if mode == 'last':
                    obuf[b] = y.astype(_BF16)
                    o_copy(b).start()
                else:
                    acc_ref[b] = y
                return [(y, r, c * 128) for c in range(D // 128) for r in range(NG)]

            def wait_group(i):
                if i == 0:
                    pl.when(step == 0)(lambda: wq_copy(0).wait())
                if i == 3:
                    pl.when(step == 0)(lambda: wo_copy(0).wait())
                for mk, j in groups[i]:
                    mk(b0 + j).wait()

            def rs(lst, n, frac=1.0):
                return [lst[int(i * len(lst) / n)] for i in range(int(n * frac))]

            if first:
                wait_group(0)
            else:
                kv_copy(kt_hbm, kbuf, ksem, step).wait()
                kv_copy(vt_hbm, vbuf, vsem, step).wait()

                @pl.when((step & 1) == 0)
                def _():
                    wq_copy(step >> 1).wait()
                    wo_copy(step >> 1).wait()

            q, qt, on, pt, o, ot = {}, {}, {}, {}, {}, {}
            q[0], qt[0] = qproj(0)
            if first:
                wait_group(1)
            for j in range(NB):
                tk = qk(j, 0, q[j][0])
                if first:
                    soft(j, 0)
                elif j > 0:
                    soft(j - 1, 1, (rs(ot[j - 2], 90) if j > 1 else []) + rs(pt[j - 1, 0], 74)
                         + rs(tk, 96, 1.0 if j + 1 < NB else _CUT))
                if j + 1 < NB:
                    q[j + 1], qt[j + 1] = qproj(j + 1)
                if j > 0:
                    on[j - 1, 1], pt[j - 1, 1] = pv(j - 1, 1)
                    o[j - 1] = [on[j - 1, 0], omid(j - 1), on[j - 1, 1]]
                tk = qk(j, 1, q[j][1])
                if first:
                    if j + 2 < len(groups):
                        wait_group(j + 2)
                    soft(j, 1)
                else:
                    soft(j, 0, (rs(qt[j + 1], 90) if j + 1 < NB else [])
                         + (rs(pt[j - 1, 1], 74) if j > 0 else []) + rs(tk, 96, 1.0 if j > 0 else _CUT))
                if j > 0:
                    ot[j - 1] = oproj(j - 1, o[j - 1])
                on[j, 0], pt[j, 0] = pv(j, 0)
            j = NB - 1
            if not first:
                soft(j, 1, rs(ot[j - 1], 90) + rs(pt[j, 0], 74, _CUT))
            on[j, 1], _ = pv(j, 1)
            oproj(j, [on[j, 0], omid(j), on[j, 1]], split=True)
            if mode == 'main':
                prefetch(step + 2)

        for b0 in (0, NB):
            for i, grp in enumerate(groups):
                if b0 == 0 and i == 0:
                    wq_copy(0).start()
                if b0 == 0 and i == 3:
                    wo_copy(0).start()
                for mk, j in grp:
                    mk(b0 + j).start()
        prefetch(2)
        prefetch(3)

        def looped(mode):
            def body(s, carry):
                run(mode, s)
                return carry
            return body

        lax.fori_loop(0, 2, looped('first'), 0)
        lax.fori_loop(2, NSTEP - 2, looped('main'), 0)
        lax.fori_loop(NSTEP - 2, NSTEP, looped('last'), 0)
        for b in range(B):
            o_copy(b).wait()

    return pl.pallas_call(
        kern,
        in_specs=[pl.BlockSpec(memory_space=pl.ANY)] * 5,
        out_specs=pl.BlockSpec(memory_space=pl.ANY),
        out_shape=jax.ShapeDtypeStruct((B, Sq, D), x.dtype),
        scratch_shapes=[
            pltpu.VMEM((B, Sq, D), _BF16),
            pltpu.VMEM((NSL * NB, W, Sk), _BF16),
            pltpu.VMEM((NSL * NB, W, Sk), _BF16),
            pltpu.VMEM((2, D, W), _BF16),
            pltpu.VMEM((2, W, D), _BF16),
            pltpu.VMEM((B, Sq, D), _BF16),
            pltpu.VMEM((B, Sq, D), _F32),
            pltpu.VMEM((1, Sq, Sk), _F32), pltpu.VMEM((1, Sq, Sk), _F32),
            pltpu.VMEM((1, Sh + Sq, Sk), _U32), pltpu.VMEM((1, Sh + Sq, Sk), _U32),
            pltpu.VMEM((4, Sq, 128), _F32),
            pltpu.VMEM((1, 128, Sq), _F32), pltpu.VMEM((1, 128, Sq), _F32),
            pltpu.SemaphoreType.DMA((44,)),
        ],
        compiler_params=pltpu.CompilerParams(
            vmem_limit_bytes=100 * 1024 * 1024,
            disable_bounds_checks=True,
            disable_semaphore_checks=True,
        ),
    )(x, kt, vt, wq, wo)
```

```python
import math

import jax
import jax.numpy as jnp
from jax import lax
import jax.experimental.pallas as pl
import jax.experimental.pallas.tpu as pltpu

_NT = (((1,), (1,)), ((), ()))
_F32 = jnp.float32
_BF16 = jnp.bfloat16
_U32 = jnp.uint32

_NB = 4
_NSL = 4
_MPACE = 3
_CUT = 0.3
_FCUT = (0.3, 0.4, 0.3)
_FSPLIT = dict(q1=(0, 128, 240), k013=(0, 64, 128, 192, 240), k113=(0, 128, 192, 240),
               k213=(0, 64, 128, 192, 240))
_TAIL = dict(first=(0, 160, 208, 240), main=(0, 128, 240), last=(0, 64, 128, 192, 240))


def _pk(v):
    return pltpu.bitcast(v, _U32)


def _upk(v):
    return pltpu.bitcast(v, _BF16)


def _dot(a, b):
    return jnp.dot(a, b, preferred_element_type=_F32)


def _dot_nt(a, b):
    return lax.dot_general(a, b, _NT, preferred_element_type=_F32)


@jax.jit
def pallas_standalone__gqa_block_cached__near_ridge_kernel(
    x: jax.Array,
    k_cache: jax.Array,
    v_cache: jax.Array,
    wq: jax.Array,
    wo: jax.Array,
):
    B, Sq, D = x.shape
    _, H, Sk, Dh = k_cache.shape
    NB, NSL = _NB, _NSL
    P = H // 2
    W = 2 * Dh
    assert B == 2 * NB and Dh == 192 and wq.shape == (D, H * Dh) and Sq == 240
    Sh = Sq // 2
    NG = Sq // 8
    NSTEP = 2 * P
    kt = jnp.swapaxes(k_cache, 2, 3).reshape(B, P, W, Sk)
    vt = jnp.swapaxes(v_cache, 2, 3).reshape(B, P, W, Sk)
    qscale = (Dh ** -0.5) * math.log2(math.e)

    def kern(x_hbm, kt_hbm, vt_hbm, wq_hbm, wo_hbm, o_hbm,
             x_ref, kbuf, vbuf, wqbuf, wobuf, obuf, acc_ref,
             s0, s1, p0, p1, r_sc, ot0, ot1, sems):
        xsem, k0sem, v0sem, wqsem, wosem, ksem, vsem, osem = 0, 8, 16, 24, 26, 28, 32, 36
        s_sc, p_sc, ot_sc = (s0, s1), (p0, p1), (ot0, ot1)
        lo = lax.broadcasted_iota(jnp.int32, (Sq, 128), 1) < 64

        def kv_copy(hbm, buf, sem, st):
            sl = st & (NSL - 1)
            return pltpu.make_async_copy(hbm.at[pl.ds((st & 1) * NB, NB), st >> 1],
                                         buf.at[pl.ds(sl * NB, NB)], sems.at[sem + sl])

        def k0_copy(b):
            return pltpu.make_async_copy(kt_hbm.at[b, 0], kbuf.at[b], sems.at[k0sem + b])

        def v0_copy(b):
            return pltpu.make_async_copy(vt_hbm.at[b, 0], vbuf.at[b], sems.at[v0sem + b])

        def x_copy(b):
            return pltpu.make_async_copy(x_hbm.at[b], x_ref.at[b], sems.at[xsem + b])

        def wq_copy(pp):
            return pltpu.make_async_copy(wq_hbm.at[:, pl.ds(pl.multiple_of(pp * W, 128), W)],
                                         wqbuf.at[pp & 1], sems.at[wqsem + (pp & 1)])

        def wo_copy(pp):
            return pltpu.make_async_copy(wo_hbm.at[pl.ds(pl.multiple_of(pp * W, 128), W), :],
                                         wobuf.at[pp & 1], sems.at[wosem + (pp & 1)])

        def o_copy(b):
            return pltpu.make_async_copy(obuf.at[b], o_hbm.at[b], sems.at[osem + b])

        def o_part(b, i):
            rows = pl.ds(_TAIL['last'][i], _TAIL['last'][i + 1] - _TAIL['last'][i])
            return pltpu.make_async_copy(obuf.at[b, rows], o_hbm.at[b, rows], sems.at[osem + b + i * B])

        groups = (((x_copy, 0), (x_copy, 1)),
                  ((k0_copy, 0), (x_copy, 2)),
                  ((v0_copy, 0), (k0_copy, 1), (x_copy, 3)),
                  ((v0_copy, 1), (k0_copy, 2)),
                  ((v0_copy, 2), (k0_copy, 3), (v0_copy, 3)))

        def on_even(st, f):
            if isinstance(st, int):
                if st % 2 == 0:
                    f()
            else:
                pl.when((st & 1) == 0)(f)

        def prefetch(st):
            on_even(st, lambda: wq_copy(st >> 1).start())
            kv_copy(kt_hbm, kbuf, ksem, st).start()
            kv_copy(vt_hbm, vbuf, vsem, st).start()
            on_even(st, lambda: wo_copy(st >> 1).start())

        def run(mode, step):
            first = mode == 'first'
            z1 = lax.shift_right_logical(step, 10)
            z2 = lax.shift_right_logical(step, 11)
            z3 = lax.shift_right_logical(step, 12)
            never = z1 > 0
            if first:
                ws, b0, kv0 = 0, step * NB, step * NB
            else:
                ws = (step >> 1) & 1
                b0 = (step & 1) * NB
                kv0 = (step & (NSL - 1)) * NB

            def rows_dot(lhs, rhs, tag):
                if first and tag in _FSPLIT:
                    c = _FSPLIT[tag]
                    return jnp.concatenate([_dot(lhs[a:b], rhs) for a, b in zip(c, c[1:])], axis=0)
                return _dot(lhs, rhs)

            def qproj(j):
                q = rows_dot(x_ref[b0 + j], wqbuf[ws], 'q%d' % j) * qscale
                q1 = q[:, 128:256]
                qa = jnp.concatenate([q[:, 0:128], jnp.where(lo, q1, 0.0)], axis=1).astype(_BF16)
                qb = jnp.concatenate([jnp.where(lo, 0.0, q1), q[:, 256:384]], axis=1).astype(_BF16)
                return (qa, qb), [(q, r, c * 128) for c in range(3) for r in range(NG)]

            def qk(j, h, q):
                ss = s_sc[h].at[z1]
                ticks = []
                for n in range(Sk // 256):
                    sv = rows_dot(q, kbuf[kv0 + j, h * 128:h * 128 + 256, n * 256:(n + 1) * 256], 'k%d%d%d' % (j, h, n))
                    ss[:, n * 256:(n + 1) * 256] = sv
                    ticks += [(sv, r, 0) for r in range(NG)]
                return ticks

            def soft(h, ticks):
                ss = s_sc[h].at[z2]
                sm = s_sc[h].at[z3]
                ps = p_sc[h].at[z1]

                def tick(g):
                    sv, r, c = ticks[int(g * len(ticks) / NG)]
                    return sv[r * 8:(r + 1) * 8, c:c + 128]

                ms = []
                for g in range(NG):
                    sv8 = sm[g * 8:(g + 1) * 8, :]
                    t0 = sv8[:, 0:128]
                    if g >= _MPACE:
                        t0 = jnp.where(never, tick(g - _MPACE), t0)
                    for t in range(1, Sk // 128):
                        t0 = jnp.maximum(t0, sv8[:, t * 128:(t + 1) * 128])
                    ms.append(jnp.max(t0, axis=1, keepdims=True))
                ls = []
                for i in range(NG // 2):
                    s = ss[i * 16:(i + 1) * 16, :]
                    es = []
                    for gi in range(2):
                        g = 2 * i + gi
                        sg = s[gi * 8:(gi + 1) * 8]
                        mb = jnp.where(never, tick(g), jnp.broadcast_to(ms[g], (8, 128)))
                        eg = jnp.concatenate(
                            [jnp.exp2(sg[:, t * 128:(t + 1) * 128] - mb) for t in range(Sk // 128)], axis=1)
                        ls.append(jnp.sum(eg, axis=1, keepdims=True))
                        es.append(eg)
                    ps[i * 8:(i + 1) * 8, :] = _pk(jnp.concatenate(es, axis=0).astype(_BF16))
                    for g in (2 * i, 2 * i + 1):
                        ps[Sh + g * 8:Sh + (g + 1) * 8, 0:128] = _pk(jnp.broadcast_to(ls[g], (8, 128)))

            def pv(j, h):
                ps = p_sc[h].at[z2]
                ot = on = None
                ticks = []
                for kc in range(Sk // 128):
                    k0, k1 = kc * 128, (kc + 1) * 128
                    a = _dot_nt(vbuf[kv0 + j, 128 + 64 * h:192 + 64 * h, k0:k1], _upk(ps[0:Sh, k0:k1]))
                    ot = a if ot is None else ot + a
                    if kc == Sk // 128 - 1:
                        ot_sc[j % 2].at[z1][h * 64:(h + 1) * 64, :] = ot
                    a = _dot_nt(_upk(ps[0:Sh, k0:k1]), vbuf[kv0 + j, 256 * h:256 * h + 128, k0:k1])
                    on = a if on is None else on + a
                    ticks += [(a, r, 0) for r in range(12)]
                rr = 1.0 / pltpu.bitcast(ps[Sh:Sh + Sq, 0:128], _F32)
                r_sc[(2 * j + h) % 4] = rr
                return on * rr, ticks

            def omid(j):
                o1 = ot_sc[j % 2].at[z2][...].T
                return o1 * jnp.where(lo, r_sc[(2 * j) % 4], r_sc[(2 * j + 1) % 4])

            def oproj(j, o):
                b = b0 + j
                y = None if first else acc_ref[b]
                yt = _dot(jnp.concatenate(o, axis=1).astype(_BF16), wobuf[ws])
                y = yt if y is None else yt + y
                if mode == 'last':
                    obuf[b] = y.astype(_BF16)
                    o_copy(b).start()
                else:
                    acc_ref[b] = y
                return [(y, r, c * 128) for c in range(D // 128) for r in range(NG)]

            def oproj_tail(j, o):
                b = b0 + j
                y = None if first else acc_ref[b]
                ob = [v.astype(_BF16) for v in o]
                y0 = _dot(ob[0], wobuf[ws, 0:128, :])
                y = y0 if first else y + y0
                cuts = _TAIL[mode]
                for i, (r0, r1) in enumerate(zip(cuts, cuts[1:])):
                    yi = y[r0:r1]
                    for t in (2, 1):
                        yi = yi + _dot(ob[t][r0:r1], wobuf[ws, t * 128:(t + 1) * 128, :])
                    if mode == 'last':
                        obuf[b, r0:r1] = yi.astype(_BF16)
                        o_part(b, i).start()
                    else:
                        acc_ref[b, r0:r1] = yi

            def wait_group(i):
                if i == 0:
                    pl.when(step == 0)(lambda: wq_copy(0).wait())
                if i == 3:
                    pl.when(step == 0)(lambda: wo_copy(0).wait())
                for mk, j in groups[i]:
                    mk(b0 + j).wait()

            def rs(lst, n, frac=1.0):
                return [lst[int(i * len(lst) / n)] for i in range(int(n * frac))]

            if first:
                wait_group(0)
            else:
                kv_copy(kt_hbm, kbuf, ksem, step).wait()
                kv_copy(vt_hbm, vbuf, vsem, step).wait()

                @pl.when((step & 1) == 0)
                def _():
                    wq_copy(step >> 1).wait()
                    wo_copy(step >> 1).wait()

            q, qt, on, pt, o, ot = {}, {}, {}, {}, {}, {}
            ahead = 2 if first else 1
            for j in range(ahead):
                q[j], qt[j] = qproj(j)
            if first:
                wait_group(1)
            for j in range(NB):
                tk = qk(j, 0, q[j][0])
                if j > 0:
                    soft(1, (rs(ot[j - 2], 90) if j > 1 else []) + rs(pt[j - 1, 0], 74)
                         + rs(tk, 96, 1.0 if j + ahead < NB else _CUT))
                if j + ahead < NB:
                    q[j + ahead], qt[j + ahead] = qproj(j + ahead)
                if j > 0:
                    on[j - 1, 1], pt[j - 1, 1] = pv(j - 1, 1)
                    o[j - 1] = [on[j - 1, 0], omid(j - 1), on[j - 1, 1]]
                tk = qk(j, 1, q[j][1])
                gate = first and j + 2 < len(groups)
                soft(0, (rs(qt[j + ahead], 90) if j + ahead < NB else [])
                     + (rs(pt[j - 1, 1], 74) if j > 0 else [])
                     + rs(tk, 96, _FCUT[j] if gate else (1.0 if j > 0 else _CUT)))
                if gate:
                    wait_group(j + 2)
                if j > 0:
                    ot[j - 1] = oproj(j - 1, o[j - 1])
                on[j, 0], pt[j, 0] = pv(j, 0)
            j = NB - 1
            soft(1, rs(ot[j - 1], 90) + rs(pt[j, 0], 74, _CUT))
            on[j, 1], _ = pv(j, 1)
            oproj_tail(j, [on[j, 0], omid(j), on[j, 1]])
            if mode == 'main':
                prefetch(step + 2)

        for b0 in (0, NB):
            for i, grp in enumerate(groups):
                if b0 == 0 and i == 0:
                    wq_copy(0).start()
                if b0 == 0 and i == 3:
                    wo_copy(0).start()
                for mk, j in grp:
                    mk(b0 + j).start()
        prefetch(2)
        prefetch(3)

        def looped(mode):
            def body(s, carry):
                run(mode, s)
                return carry
            return body

        lax.fori_loop(0, 2, looped('first'), 0)
        lax.fori_loop(2, NSTEP - 2, looped('main'), 0)
        lax.fori_loop(NSTEP - 2, NSTEP, looped('last'), 0)
        for b in range(B):
            if b % NB == NB - 1:
                for i in range(len(_TAIL['last']) - 1):
                    o_part(b, i).wait()
            else:
                o_copy(b).wait()

    return pl.pallas_call(
        kern,
        in_specs=[pl.BlockSpec(memory_space=pl.ANY)] * 5,
        out_specs=pl.BlockSpec(memory_space=pl.ANY),
        out_shape=jax.ShapeDtypeStruct((B, Sq, D), x.dtype),
        scratch_shapes=[
            pltpu.VMEM((B, Sq, D), _BF16),
            pltpu.VMEM((NSL * NB, W, Sk), _BF16),
            pltpu.VMEM((NSL * NB, W, Sk), _BF16),
            pltpu.VMEM((2, D, W), _BF16),
            pltpu.VMEM((2, W, D), _BF16),
            pltpu.VMEM((B, Sq, D), _BF16),
            pltpu.VMEM((B, Sq, D), _F32),
            pltpu.VMEM((1, Sq, Sk), _F32), pltpu.VMEM((1, Sq, Sk), _F32),
            pltpu.VMEM((1, Sh + Sq, Sk), _U32), pltpu.VMEM((1, Sh + Sq, Sk), _U32),
            pltpu.VMEM((4, Sq, 128), _F32),
            pltpu.VMEM((1, 128, Sq), _F32), pltpu.VMEM((1, 128, Sq), _F32),
            pltpu.SemaphoreType.DMA((68,)),
        ],
        compiler_params=pltpu.CompilerParams(
            vmem_limit_bytes=100 * 1024 * 1024,
            disable_bounds_checks=True,
            disable_semaphore_checks=True,
        ),
    )(x, kt, vt, wq, wo)
```
